```python
import os as _os
_os.environ.setdefault("JAX_PLATFORMS", "cpu")
import jax
import jax.numpy as jnp

def _softmax(x, axis=-1):
    return jax.nn.softmax(x, axis=axis)
def _gelu(x):
    return jax.nn.gelu(x, approximate=True)
def _silu(x):
    return jax.nn.silu(x)
def _sigmoid(x):
    return jax.nn.sigmoid(x)
def _layernorm(x, axis=-1, eps=1e-5):
    m = jnp.mean(x, axis=axis, keepdims=True)
    v = jnp.var(x, axis=axis, keepdims=True)
    return (x - m) / jnp.sqrt(v + eps)
def _scatter_add(tgt, idx, src, axis=0):
    return tgt.at[idx].add(src)
def _segment_sum(src, seg, n):
    return jax.ops.segment_sum(src, seg, n)
class _Rng:
    def __init__(self, key):
        self._k = key
    def _next(self):
        self._k, sub = jax.random.split(self._k)
        return sub
    def normal(self, shape):
        return jax.random.normal(self._next(), shape, dtype=jnp.bfloat16)
    def randint(self, lo, hi, shape):
        return jax.random.randint(self._next(), shape, lo, hi, dtype=jnp.int32)
    def uniform(self, shape, lo=0.0, hi=1.0):
        return jax.random.uniform(self._next(), shape, jnp.bfloat16, lo, hi)
    def permutation(self, n):
        return jax.random.permutation(self._next(), n)


kernel_name = 'concat_heads__mha_block_cached__gqa_block_cached__near_ridge'

def setup_inputs():
    _rng = _Rng(jax.random.key(int.from_bytes(__import__("os").urandom(4), "little")))
    _w = (lambda a: (lambda t: t.astype(jnp.bfloat16) if jnp.issubdtype(t.dtype, jnp.floating) else t)(jnp.asarray(a)))
    def _A_setup():
        B, Sq, D = 8, 128, 640
        H, Sk, Dh = 32, 1024, 192
        return {
            "x": _w((lambda *s: _rng.normal(s) * 0.8)(B, Sq, D)),
            "k_cache": _w((lambda *s: _rng.normal(s) * 0.8)(B, H, Sk, Dh)),
            "v_cache": _w((lambda *s: _rng.normal(s) * 0.05)(B, H, Sk, Dh)),
            "wq": _w((lambda *s: _rng.normal(s) * 0.8)(D, H * Dh) * (D ** -0.5)),
            "wo": _w((lambda *s: _rng.normal(s) * 0.05)(H * Dh, D) * ((H * Dh) ** -0.5)),
        }
    _A_in = _A_setup()

    def _B_setup():
        B, Sq, D = 8, 128, 640
        Hq, Hkv, Sk, Dh = 32, 32, 1024, 192
        assert Hq % Hkv == 0, (Hq, Hkv)
        return {
            "x": _w((lambda *s: _rng.normal(s) * 0.8)(B, Sq, D)),
            "k_cache": _w((lambda *s: _rng.normal(s) * 0.8)(B, Hkv, Sk, Dh)),
            "v_cache": _w((lambda *s: _rng.normal(s) * 0.05)(B, Hkv, Sk, Dh)),
            "wq": _w((lambda *s: _rng.normal(s) * 0.8)(D, Hq * Dh) * (D ** -0.5)),
            "wo": _w((lambda *s: _rng.normal(s) * 0.05)(Hq * Dh, D) * ((Hq * Dh) ** -0.5)),
        }
    _B_in = _B_setup()

    return {
        "A_x": _A_in["x"],
        "A_k_cache": _A_in["k_cache"],
        "A_v_cache": _A_in["v_cache"],
        "A_wq": _A_in["wq"],
        "A_wo": _A_in["wo"],
        "B_x": _B_in["x"],
        "B_k_cache": _B_in["k_cache"],
        "B_v_cache": _B_in["v_cache"],
        "B_wq": _B_in["wq"],
        "B_wo": _B_in["wo"],
    }

def reference(A_x, A_k_cache, A_v_cache, A_wq, A_wo, B_x, B_k_cache, B_v_cache, B_wq, B_wo):
    def _A_ref(x, k_cache, v_cache, wq, wo):
        B, Sq, D = x.shape
        H, Dh = 32, 192
        q = (lambda x, *d: x.transpose(*d))((x @ wq).reshape(B, Sq, H, Dh), 0, 2, 1, 3)
        scores = jnp.einsum("bhqd,bhkd->bhqk", q, k_cache) * (Dh ** -0.5)
        p = _softmax(scores, axis=-1)
        o = jnp.einsum("bhqk,bhkd->bhqd", p, v_cache)
        return (lambda x, *d: x.transpose(*d))(o, 0, 2, 1, 3).reshape(B, Sq, H * Dh) @ wo

    def _B_ref(x, k_cache, v_cache, wq, wo):
        B, Sq, D = x.shape
        Hq, Dh = 32, 192
        Hkv = k_cache.shape[1]
        rep = Hq // Hkv
        q = (lambda x, *d: x.transpose(*d))((x @ wq).reshape(B, Sq, Hq, Dh), 0, 2, 1, 3)
        k = jnp.repeat(k_cache, rep, axis=1)
        v = jnp.repeat(v_cache, rep, axis=1)
        scores = jnp.einsum("bhqd,bhkd->bhqk", q, k) * (Dh ** -0.5)
        p = _softmax(scores, axis=-1)
        o = jnp.einsum("bhqk,bhkd->bhqd", p, v)
        return (lambda x, *d: x.transpose(*d))(o, 0, 2, 1, 3).reshape(B, Sq, Hq * Dh) @ wo

    a = _A_ref(A_x, A_k_cache, A_v_cache, A_wq, A_wo)
    b = _B_ref(B_x, B_k_cache, B_v_cache, B_wq, B_wo)
    return jnp.concatenate([a, b], axis=-1)
```

```python
import math
import jax
import jax.numpy as jnp
from jax import lax
import jax.experimental.pallas as pl
import jax.experimental.pallas.tpu as pltpu

B, SQ, D = 8, 128, 640
H, SK, DH = 32, 1024, 192
HP = H // 2
P2 = 2 * DH
NSTEP = HP * B
NBUF = 4
QSCALE = (DH ** -0.5) * math.log2(math.e)
NT = (((1,), (1,)), ((), ()))
F32 = jnp.float32
BF16 = jnp.bfloat16


def _kernel(xa, xb, wqa, wqb, woa, wob, kta, vta, ktb, vtb, o_hbm,
            x_v, wq_v, wo_v, kv_v, q_v, acc_v, wot_v, out_v, sem_kv, sem_w, sem_x, sem_o):
    kv_hbm = (kta, vta, ktb, vtb)

    def kv_copy(t, j):
        slot = t % NBUF
        return pltpu.make_async_copy(kv_hbm[j].at[t % B, t // B], kv_v.at[slot, j], sem_kv.at[slot, j])

    def wq_copy(hp, br):
        src = (wqa, wqb)[br]
        return pltpu.make_async_copy(src.at[:, pl.ds(pl.multiple_of(hp * P2, 128), P2)], wq_v.at[hp % 2, br],
                                     sem_w.at[hp % 2, br])

    def wo_copy(hp, br):
        src = (woa, wob)[br]
        return pltpu.make_async_copy(src.at[pl.ds(pl.multiple_of(hp * P2, 128), P2), :], wo_v.at[hp % 2, br],
                                     sem_w.at[hp % 2, 2 + br])

    def x_copy(br):
        return pltpu.make_async_copy((xa, xb)[br], x_v.at[br], sem_x.at[br])

    def o_copy(b):
        return pltpu.make_async_copy(out_v.at[b], o_hbm.at[b], sem_o.at[b])

    lane = lax.broadcasted_iota(jnp.int32, (SQ, 128), 1) < 64
    ones = jnp.ones((16, SK), BF16)

    def qproj(br, b, hp):
        q = jnp.dot(x_v[br, b], wq_v[hp % 2, br], preferred_element_type=F32) * QSCALE
        t0, t1, t2 = q[:, :128], q[:, 128:256], q[:, 256:]
        q_v[br, 0] = jnp.concatenate([t0, jnp.where(lane, t1, 0.0)], axis=1).astype(BF16)
        q_v[br, 1] = jnp.concatenate([jnp.where(lane, 0.0, t1), t2], axis=1).astype(BF16)

    for br in range(2):
        x_copy(br).start()
        wq_copy(0, br).start()
    for j in range(4):
        kv_copy(0, j).start()
    for br in range(2):
        wo_copy(0, br).start()
    for t in range(1, NBUF - 1):
        for j in range(4):
            kv_copy(t, j).start()
    acc_v[...] = jnp.zeros(acc_v.shape, F32)
    for br in range(2):
        x_copy(br).wait()
        wq_copy(0, br).wait()
    qproj(0, 0, 0)
    qproj(1, 0, 0)

    def step(t, carry):
        hp = t // B
        b = t % B
        slot = t % NBUF

        @pl.when(t + NBUF - 1 < NSTEP)
        def _():
            for j in range(4):
                kv_copy(t + NBUF - 1, j).start()

        @pl.when(b == 0)
        def _():
            @pl.when(hp + 1 < HP)
            def _():
                for br in range(2):
                    wq_copy(hp + 1, br).start()
                for br in range(2):
                    wo_copy(hp + 1, br).start()
            for br in range(2):
                wo_copy(hp, br).wait()
                wot_v[br] = wo_v[hp % 2, br].T

        @pl.when(jnp.logical_and(b == B - 1, hp + 1 < HP))
        def _():
            for br in range(2):
                wq_copy(hp + 1, br).wait()

        for j in range(4):
            kv_copy(t, j).wait()

        tn = jnp.minimum(t + 1, NSTEP - 1)
        hpn = tn // B
        bn = tn % B

        def qk(br, hh):
            return jnp.dot(q_v[br, hh], kv_v[slot, 2 * br, pl.ds(hh * 128, 256), :], preferred_element_type=F32)

        def sm(s):
            m = jnp.max(s, axis=1, keepdims=True)
            return jnp.exp2(s - m).astype(BF16)

        def pv(p, br, hh):
            va = jnp.concatenate([kv_v[slot, 2 * br + 1, pl.ds(hh * DH, DH), :], ones], axis=0)
            ot = lax.dot_general(va, p, NT, preferred_element_type=F32)
            inv = 1.0 / ot[DH:DH + 1, :]
            return (ot[:DH] * inv).astype(BF16)

        def oproj(br, o1, o2):
            otp = jnp.concatenate([o1, o2], axis=0)
            acc_v[b, br] += jnp.dot(wot_v[br], otp, preferred_element_type=F32)

        sa1 = qk(0, 0)
        sa2 = qk(0, 1)
        oa1 = pv(sm(sa1), 0, 0)
        sb1 = qk(1, 0)
        oa2 = pv(sm(sa2), 0, 1)
        sb2 = qk(1, 1)
        ob1 = pv(sm(sb1), 1, 0)
        oproj(0, oa1, oa2)
        ob2 = pv(sm(sb2), 1, 1)
        qproj(0, bn, hpn)
        oproj(1, ob1, ob2)
        qproj(1, bn, hpn)

        @pl.when(hp == HP - 1)
        def _():
            out_v[b, :, 0:D] = acc_v[b, 0].T.astype(BF16)
            out_v[b, :, D:2 * D] = acc_v[b, 1].T.astype(BF16)
            o_copy(b).start()

        return carry

    lax.fori_loop(0, NSTEP, step, 0)
    for b in range(B):
        o_copy(b).wait()


@jax.jit
def pallas_concat_heads__mha_block_cached__gqa_block_cached__near_ridge_kernel(
    A_x, A_k_cache, A_v_cache, A_wq, A_wo, B_x, B_k_cache, B_v_cache, B_wq, B_wo):
    t = lambda z: jnp.swapaxes(z, 2, 3).reshape(B, HP, P2, SK)
    any_spec = pl.BlockSpec(memory_space=pl.ANY)
    return pl.pallas_call(
        _kernel,
        in_specs=[any_spec] * 10,
        out_specs=any_spec,
        out_shape=jax.ShapeDtypeStruct((B, SQ, 2 * D), BF16),
        scratch_shapes=[
            pltpu.VMEM((2, B, SQ, D), BF16),
            pltpu.VMEM((2, 2, D, P2), BF16),
            pltpu.VMEM((2, 2, P2, D), BF16),
            pltpu.VMEM((NBUF, 4, P2, SK), BF16),
            pltpu.VMEM((2, 2, SQ, 256), BF16),
            pltpu.VMEM((B, 2, D, SQ), F32),
            pltpu.VMEM((2, D, P2), BF16),
            pltpu.VMEM((B, SQ, 2 * D), BF16),
            pltpu.SemaphoreType.DMA((NBUF, 4)),
            pltpu.SemaphoreType.DMA((2, 4)),
            pltpu.SemaphoreType.DMA((2,)),
            pltpu.SemaphoreType.DMA((B,)),
        ],
        compiler_params=pltpu.CompilerParams(vmem_limit_bytes=64 * 1024 * 1024),
    )(A_x, B_x, A_wq, B_wq, A_wo, B_wo, t(A_k_cache), t(A_v_cache), t(B_k_cache), t(B_v_cache))
```

```python
import math
import jax
import jax.numpy as jnp
from jax import lax
import jax.experimental.pallas as pl
import jax.experimental.pallas.tpu as pltpu

B, SQ, D = 8, 128, 640
H, SK, DH = 32, 1024, 192
HP = H // 2
P2 = 2 * DH
NSTEP = HP * B
NBUF = 4
GROUP = (40, 24)
GR = sum(GROUP)
NG = P2 // GR
KOFF = 2
VOFF = 2
WQ_ROWS = D // B
WO_ROWS = P2 // B
QSCALE = (DH ** -0.5) * math.log2(math.e)
NT = (((1,), (1,)), ((), ()))
F32 = jnp.float32
BF16 = jnp.bfloat16


def _kernel(xa, xb, wqa, wqb, woa, wob, kta, vta, ktb, vtb, o_hbm,
            x_v, wq_v, wo_v, kv_v, q_v, acc_v, out_v, sem_kv, sem_w, sem_x, sem_o):
    kv_hbm = (kta, vta, ktb, vtb)

    def start(cp, prio):
        src, dst, sem = cp
        pltpu.make_async_copy(src, dst, sem).start(priority=prio)

    def issue(copies):
        for n, cp in enumerate(copies):
            start(cp, n % 2)

    def issue2(p0, p1):
        for n in range(max(len(p0), len(p1))):
            if n < len(p0):
                start(p0[n], 0)
            if n < len(p1):
                start(p1[n], 1)

    def wait_all(buf, sem):
        pltpu.make_async_copy(buf, buf, sem).wait()

    def kv_groups(t, kind, g0, g1):
        slot = t % NBUF
        tb = t % B
        th = t // B
        out = []
        for g in range(g0, g1):
            r = g * GR
            for sz in GROUP:
                for br in range(2):
                    j = 2 * br + kind
                    out.append((kv_hbm[j].at[tb, th, pl.ds(r, sz)], kv_v.at[slot, j, pl.ds(r, sz)],
                                sem_kv.at[slot, j]))
                r += sz
        return out

    def wq_pieces(hp, j):
        c0 = pl.multiple_of(hp * P2, 128)
        rq = pl.multiple_of(j * WQ_ROWS, 16)
        return [((wqa, wqb)[br].at[pl.ds(rq, WQ_ROWS), pl.ds(c0, P2)], wq_v.at[hp, br, pl.ds(rq, WQ_ROWS)],
                 sem_w.at[hp % 2, br]) for br in range(2)]

    def wo_pieces(hp, j):
        ro = pl.multiple_of(j * WO_ROWS, 16)
        r0 = pl.multiple_of(hp * P2 + j * WO_ROWS, 16)
        return [((woa, wob)[br].at[pl.ds(r0, WO_ROWS)], wo_v.at[hp, br, pl.ds(ro, WO_ROWS)],
                 sem_w.at[hp % 2, 2 + br]) for br in range(2)]

    def o_copy(b):
        return pltpu.make_async_copy(out_v.at[b], o_hbm.at[b], sem_o.at[b])

    lane = lax.broadcasted_iota(jnp.int32, (SQ, 128), 1) < 64
    ones = jnp.ones((16, SK), BF16)

    def qproj(br, b, hp):
        q = jnp.dot(x_v[br, b], wq_v[hp, br], preferred_element_type=F32) * QSCALE
        t0, t1, t2 = q[:, :128], q[:, 128:256], q[:, 256:]
        q_v[b, br, 0] = jnp.concatenate([t0, jnp.where(lane, t1, 0.0)], axis=1).astype(BF16)
        q_v[b, br, 1] = jnp.concatenate([jnp.where(lane, 0.0, t1), t2], axis=1).astype(BF16)

    def qk(slot, b, br, hh):
        return jnp.dot(q_v[b, br, hh], kv_v[slot, 2 * br, pl.ds(hh * 128, 256), :], preferred_element_type=F32)

    def sm(s):
        m = jnp.max(s, axis=1, keepdims=True)
        return jnp.exp2(s - m).astype(BF16)

    def pv(slot, p, br, hh):
        va = jnp.concatenate([kv_v[slot, 2 * br + 1, pl.ds(hh * DH, DH), :], ones], axis=0)
        ot = lax.dot_general(va, p, NT, preferred_element_type=F32)
        inv = 1.0 / ot[DH:DH + 1, :]
        return (ot[:DH] * inv).astype(BF16)

    def oproj(b, hp, br, o1, o2):
        op = jnp.concatenate([o1, o2], axis=0).T
        acc_v[b, br] += jnp.dot(op, wo_v[hp, br], preferred_element_type=F32)

    def oproj_final(b, hp, br, o1, o2):
        op = jnp.concatenate([o1, o2], axis=0).T
        r = acc_v[b, br] + jnp.dot(op, wo_v[hp, br], preferred_element_type=F32)
        out_v[b, :, pl.ds(br * D, D)] = r.astype(BF16)

    def new_head_pair(hp):
        for br in range(2):
            wait_all(wo_v.at[hp, br], sem_w.at[hp % 2, 2 + br])

    cps = []
    for b in range(B):
        for r in range(0, SQ, 32):
            for br in range(2):
                cps.append(((xa, xb)[br].at[b, pl.ds(r, 32)], x_v.at[br, b, pl.ds(r, 32)], sem_x.at[br]))
        if b == 0:
            for j in range(B):
                cps += wq_pieces(0, j)
    issue(cps)
    p0 = []
    for j in range(B):
        p0 += wo_pieces(0, j) + wq_pieces(1, j)
    issue2(p0[:24], kv_groups(0, 1, 0, NG))
    acc_v[...] = jnp.zeros(acc_v.shape, F32)
    for br in range(2):
        wait_all(x_v.at[br], sem_x.at[br])
        wait_all(wq_v.at[0, br], sem_w.at[0, br])
    issue2(p0[24:] + kv_groups(0, 0, 0, NG) + kv_groups(1, 0, 0, KOFF),
           kv_groups(1, 1, 0, NG) + kv_groups(2, 1, 0, VOFF))
    for t in range(NBUF - 1):
        issue(wq_pieces(2, t) + wo_pieces(1, t))

    def q0(b, carry):
        qproj(0, b, 0)
        qproj(1, b, 0)
        return carry

    lax.fori_loop(0, B, q0, 0)
    issue2(kv_groups(1, 0, KOFF, NG) + kv_groups(2, 0, 0, KOFF),
           kv_groups(2, 1, VOFF, NG) + kv_groups(3, 1, 0, VOFF))

    def step(t, carry):
        hp = t // B
        b = t % B
        slot = t % NBUF
        tp = t + NBUF - 1

        @pl.when(tp < NSTEP - 2 * B)
        def _():
            issue(wq_pieces(tp // B + 2, tp % B))

        @pl.when(tp < NSTEP - B)
        def _():
            issue(wo_pieces(tp // B + 1, tp % B))

        @pl.when(b == 0)
        def _():
            for br in range(2):
                wait_all(wq_v.at[hp + 1, br], sem_w.at[(hp + 1) % 2, br])
            new_head_pair(hp)

        for j in range(4):
            wait_all(kv_v.at[slot, j], sem_kv.at[slot, j])

        sa1 = qk(slot, b, 0, 0)
        sa2 = qk(slot, b, 0, 1)
        oa1 = pv(slot, sm(sa1), 0, 0)
        sb1 = qk(slot, b, 1, 0)
        oa2 = pv(slot, sm(sa2), 0, 1)
        sb2 = qk(slot, b, 1, 1)
        ob1 = pv(slot, sm(sb1), 1, 0)
        oproj(b, hp, 0, oa1, oa2)
        ob2 = pv(slot, sm(sb2), 1, 1)
        issue2(kv_groups(t + 2, 0, KOFF, NG) + kv_groups(t + 3, 0, 0, KOFF),
               kv_groups(t + 3, 1, VOFF, NG) + kv_groups(t + 4, 1, 0, VOFF))
        qproj(0, b, hp + 1)
        oproj(b, hp, 1, ob1, ob2)
        qproj(1, b, hp + 1)
        return carry

    lax.fori_loop(0, NSTEP - B, step, 0)

    new_head_pair(HP - 1)

    def tail_step(t, carry):
        b = t % B
        slot = t % NBUF

        @pl.when(t == NSTEP - 1)
        def _():
            for bb in range(B - 1):
                o_copy(bb).start(priority=1)

        for j in range(4):
            wait_all(kv_v.at[slot, j], sem_kv.at[slot, j])

        sa1 = qk(slot, b, 0, 0)
        sa2 = qk(slot, b, 0, 1)
        oa1 = pv(slot, sm(sa1), 0, 0)
        sb1 = qk(slot, b, 1, 0)
        oa2 = pv(slot, sm(sa2), 0, 1)
        sb2 = qk(slot, b, 1, 1)
        ob1 = pv(slot, sm(sb1), 1, 0)
        oproj_final(b, HP - 1, 0, oa1, oa2)
        ob2 = pv(slot, sm(sb2), 1, 1)
        oproj_final(b, HP - 1, 1, ob1, ob2)

        @pl.when(t + 4 < NSTEP)
        def _():
            issue2(kv_groups(t + 2, 0, KOFF, NG) + kv_groups(t + 3, 0, 0, KOFF),
                   kv_groups(t + 3, 1, VOFF, NG) + kv_groups(t + 4, 1, 0, VOFF))

        @pl.when(t + 4 == NSTEP)
        def _():
            issue2(kv_groups(NSTEP - 2, 0, KOFF, NG) + kv_groups(NSTEP - 1, 0, 0, KOFF),
                   kv_groups(NSTEP - 1, 1, VOFF, NG))

        @pl.when(t + 3 == NSTEP)
        def _():
            issue2([], kv_groups(NSTEP - 1, 0, KOFF, NG))
        return carry

    lax.fori_loop(NSTEP - B, NSTEP, tail_step, 0)

    o_copy(B - 1).start()
    for b in range(B):
        o_copy(b).wait()


@jax.jit
def pallas_concat_heads__mha_block_cached__gqa_block_cached__near_ridge_kernel(
    A_x, A_k_cache, A_v_cache, A_wq, A_wo, B_x, B_k_cache, B_v_cache, B_wq, B_wo):
    t = lambda z: jnp.swapaxes(z, 2, 3).reshape(B, HP, P2, SK)
    any_spec = pl.BlockSpec(memory_space=pl.ANY)
    return pl.pallas_call(
        _kernel,
        in_specs=[any_spec] * 10,
        out_specs=any_spec,
        out_shape=jax.ShapeDtypeStruct((B, SQ, 2 * D), BF16),
        scratch_shapes=[
            pltpu.VMEM((2, B, SQ, D), BF16),
            pltpu.VMEM((HP, 2, D, P2), BF16),
            pltpu.VMEM((HP, 2, P2, D), BF16),
            pltpu.VMEM((NBUF, 4, P2, SK), BF16),
            pltpu.VMEM((B, 2, 2, SQ, 256), BF16),
            pltpu.VMEM((B, 2, SQ, D), F32),
            pltpu.VMEM((B, SQ, 2 * D), BF16),
            pltpu.SemaphoreType.DMA((NBUF, 4)),
            pltpu.SemaphoreType.DMA((2, 4)),
            pltpu.SemaphoreType.DMA((2,)),
            pltpu.SemaphoreType.DMA((B,)),
        ],
        compiler_params=pltpu.CompilerParams(vmem_limit_bytes=96 * 1024 * 1024, disable_bounds_checks=True),
    )(A_x, B_x, A_wq, B_wq, A_wo, B_wo, t(A_k_cache), t(A_v_cache), t(B_k_cache), t(B_v_cache))
```

```python
import math
import jax
import jax.numpy as jnp
from jax import lax
import jax.experimental.pallas as pl
import jax.experimental.pallas.tpu as pltpu

B, SQ, D = 8, 128, 640
H, SK, DH = 32, 1024, 192
HP = H // 2
P2 = 2 * DH
NSTEP = HP * B
NBUF = 4
PIECES = []
for _i in range(12):
    PIECES.append((0, 16) if _i == 0 else (32 * _i + 8, 8))
    PIECES.append((32 * _i + 16, 24 if _i < 11 else 16))
NPC = len(PIECES)
NCH = NPC // 2
PRE = 6
LAG = 8
WQ_ROWS = D // B
WO_ROWS = P2 // B
QSCALE = (DH ** -0.5) * math.log2(math.e)
NT = (((1,), (1,)), ((), ()))
F32 = jnp.float32
BF16 = jnp.bfloat16


def _kernel(xa, xb, wqa, wqb, woa, wob, kta, vta, ktb, vtb, o_hbm,
            x_v, wq_v, wo_v, kv_v, q_v, acc_v, out_v, sem_kv, sem_w, sem_x, sem_o):
    kv_hbm = (kta, vta, ktb, vtb)

    def start(cp, prio):
        src, dst, sem = cp
        pltpu.make_async_copy(src, dst, sem).start(priority=prio)

    def issue(copies):
        for n, cp in enumerate(copies):
            start(cp, n % 2)

    def wait_all(buf, sem):
        pltpu.make_async_copy(buf, buf, sem).wait()

    def kv_piece(t, p):
        slot = t % NBUF
        tb = t % B
        th = t // B
        r, sz = PIECES[p]
        return [(kv_hbm[j].at[tb, th, pl.ds(r, sz)], kv_v.at[slot, j, pl.ds(r, sz)], sem_kv.at[slot, j])
                for j in range(4)]

    def pair(p0, p1):
        for n in range(max(len(p0), len(p1))):
            if n < len(p0):
                start(p0[n], 0)
            if n < len(p1):
                start(p1[n], 1)

    def kv_chunk(t, c):
        pair(kv_piece(t, NCH + c), kv_piece(t, c))

    def wq_pieces(hp, j):
        c0 = pl.multiple_of(hp * P2, 128)
        rq = pl.multiple_of(j * WQ_ROWS, 16)
        return [((wqa, wqb)[br].at[pl.ds(rq, WQ_ROWS), pl.ds(c0, P2)], wq_v.at[hp, br, pl.ds(rq, WQ_ROWS)],
                 sem_w.at[hp % 2, br]) for br in range(2)]

    def wo_pieces(hp, j):
        ro = pl.multiple_of(j * WO_ROWS, 16)
        r0 = pl.multiple_of(hp * P2 + j * WO_ROWS, 16)
        return [((woa, wob)[br].at[pl.ds(r0, WO_ROWS)], wo_v.at[hp, br, pl.ds(ro, WO_ROWS)],
                 sem_w.at[hp % 2, 2 + br]) for br in range(2)]

    def o_copy(b):
        return pltpu.make_async_copy(out_v.at[b], o_hbm.at[b], sem_o.at[b])

    lane = lax.broadcasted_iota(jnp.int32, (SQ, 128), 1) < 64
    ones = jnp.ones((16, SK), BF16)

    def qproj(br, b, hp):
        q = jnp.dot(x_v[br, b], wq_v[hp, br], preferred_element_type=F32) * QSCALE
        t0, t1, t2 = q[:, :128], q[:, 128:256], q[:, 256:]
        q_v[b, br, 0] = jnp.concatenate([t0, jnp.where(lane, t1, 0.0)], axis=1).astype(BF16)
        q_v[b, br, 1] = jnp.concatenate([jnp.where(lane, 0.0, t1), t2], axis=1).astype(BF16)

    def qk(slot, b, br, hh):
        return jnp.dot(q_v[b, br, hh], kv_v[slot, 2 * br, pl.ds(hh * 128, 256), :], preferred_element_type=F32)

    def sm(s):
        m = jnp.max(s, axis=1, keepdims=True)
        return jnp.exp2(s - m).astype(BF16)

    def pv(slot, p, br, hh):
        va = jnp.concatenate([kv_v[slot, 2 * br + 1, pl.ds(hh * DH, DH), :], ones], axis=0)
        ot = lax.dot_general(va, p, NT, preferred_element_type=F32)
        inv = 1.0 / ot[DH:DH + 1, :]
        return (ot[:DH] * inv).astype(BF16)

    def oproj(b, hp, br, o1, o2):
        op = jnp.concatenate([o1, o2], axis=0).T
        acc_v[b, br] += jnp.dot(op, wo_v[hp, br], preferred_element_type=F32)

    def oproj_final(b, hp, br, o1, o2):
        op = jnp.concatenate([o1, o2], axis=0).T
        r = acc_v[b, br] + jnp.dot(op, wo_v[hp, br], preferred_element_type=F32)
        out_v[b, :, pl.ds(br * D, D)] = r.astype(BF16)

    def wait_wo(hp):
        for br in range(2):
            wait_all(wo_v.at[hp, br], sem_w.at[hp % 2, 2 + br])

    cps = []
    for b in range(B):
        for r in range(0, SQ, 32):
            for br in range(2):
                cps.append(((xa, xb)[br].at[b, pl.ds(r, 32)], x_v.at[br, b, pl.ds(r, 32)], sem_x.at[br]))
        if b == 0:
            for j in range(B):
                cps += wq_pieces(0, j)
    for j in range(B):
        cps += wo_pieces(0, j)
    for j in range(B):
        cps += wq_pieces(1, j)
    issue(cps)
    acc_v[...] = jnp.zeros(acc_v.shape, F32)
    for c in range(PRE):
        kv_chunk(0, c)
    for br in range(2):
        wait_all(x_v.at[br], sem_x.at[br])
        wait_all(wq_v.at[0, br], sem_w.at[0, br])

    def q0(b, carry):
        qproj(0, b, 0)
        qproj(1, b, 0)
        for k in range(B):
            @pl.when(b == k)
            def _():
                for c in range(PRE + 2 * k, PRE + 2 * k + 2):
                    kv_chunk(c // NCH, c % NCH)
                if k < NBUF - 1:
                    issue(wq_pieces(2, k) + wo_pieces(1, k))
        return carry

    lax.fori_loop(0, B, q0, 0)
    for c in range(PRE + 2 * B, 2 * NCH):
        kv_chunk(c // NCH, c % NCH)

    def step(t, carry):
        hp = t // B
        b = t % B
        slot = t % NBUF
        tp = t + NBUF - 1

        @pl.when(tp < NSTEP - 2 * B)
        def _():
            issue(wq_pieces(tp // B + 2, tp % B))

        @pl.when(tp < NSTEP - B)
        def _():
            issue(wo_pieces(tp // B + 1, tp % B))

        @pl.when(b == 0)
        def _():
            for br in range(2):
                wait_all(wq_v.at[hp + 1, br], sem_w.at[(hp + 1) % 2, br])
            wait_wo(hp)

        for j in range(4):
            wait_all(kv_v.at[slot, j], sem_kv.at[slot, j])

        def chunk(c):
            kv_chunk(t + 2, c)

        sa1 = qk(slot, b, 0, 0)
        chunk(0)
        sa2 = qk(slot, b, 0, 1)
        chunk(1)
        oa1 = pv(slot, sm(sa1), 0, 0)
        chunk(2)
        sb1 = qk(slot, b, 1, 0)
        chunk(3)
        oa2 = pv(slot, sm(sa2), 0, 1)
        chunk(4)
        sb2 = qk(slot, b, 1, 1)
        chunk(5)
        ob1 = pv(slot, sm(sb1), 1, 0)
        chunk(6)
        oproj(b, hp, 0, oa1, oa2)
        chunk(7)
        ob2 = pv(slot, sm(sb2), 1, 1)
        chunk(8)
        qproj(0, b, hp + 1)
        chunk(9)
        oproj(b, hp, 1, ob1, ob2)
        chunk(10)
        qproj(1, b, hp + 1)
        chunk(11)
        return carry

    lax.fori_loop(0, NSTEP - B, step, 0)

    wait_wo(HP - 1)

    def tail_step(t, carry):
        b = t % B
        slot = t % NBUF

        @pl.when(t == NSTEP - 1)
        def _():
            for bb in range(B - 1):
                o_copy(bb).start(priority=1)

        for j in range(4):
            wait_all(kv_v.at[slot, j], sem_kv.at[slot, j])

        def chunk(c):
            if c >= LAG:
                @pl.when(t + 2 < NSTEP)
                def _():
                    pair(kv_piece(t + 2, NCH + c - LAG), kv_piece(t + 2, c))
            else:
                p0 = kv_piece(t + 1, 2 * NCH + c - LAG)
                p1 = kv_piece(t + 2, c)
                for n in range(4):
                    @pl.when(jnp.logical_and(t > NSTEP - B, t + 1 < NSTEP))
                    def _():
                        start(p0[n], 0)

                    @pl.when(t + 2 < NSTEP)
                    def _():
                        start(p1[n], 1)

        sa1 = qk(slot, b, 0, 0)
        chunk(0)
        sa2 = qk(slot, b, 0, 1)
        chunk(1)
        oa1 = pv(slot, sm(sa1), 0, 0)
        chunk(2)
        sb1 = qk(slot, b, 1, 0)
        chunk(3)
        chunk(4)
        oa2 = pv(slot, sm(sa2), 0, 1)
        chunk(5)
        sb2 = qk(slot, b, 1, 1)
        chunk(6)
        ob1 = pv(slot, sm(sb1), 1, 0)
        chunk(7)
        chunk(8)
        oproj_final(b, HP - 1, 0, oa1, oa2)
        chunk(9)
        ob2 = pv(slot, sm(sb2), 1, 1)
        chunk(10)
        chunk(11)
        oproj_final(b, HP - 1, 1, ob1, ob2)
        return carry

    lax.fori_loop(NSTEP - B, NSTEP, tail_step, 0)

    o_copy(B - 1).start()
    for b in range(B):
        o_copy(b).wait()


@jax.jit
def pallas_concat_heads__mha_block_cached__gqa_block_cached__near_ridge_kernel(
    A_x, A_k_cache, A_v_cache, A_wq, A_wo, B_x, B_k_cache, B_v_cache, B_wq, B_wo):
    t = lambda z: jnp.swapaxes(z, 2, 3).reshape(B, HP, P2, SK)
    any_spec = pl.BlockSpec(memory_space=pl.ANY)
    return pl.pallas_call(
        _kernel,
        in_specs=[any_spec] * 10,
        out_specs=any_spec,
        out_shape=jax.ShapeDtypeStruct((B, SQ, 2 * D), BF16),
        scratch_shapes=[
            pltpu.VMEM((2, B, SQ, D), BF16),
            pltpu.VMEM((HP, 2, D, P2), BF16),
            pltpu.VMEM((HP, 2, P2, D), BF16),
            pltpu.VMEM((NBUF, 4, P2, SK), BF16),
            pltpu.VMEM((B, 2, 2, SQ, 256), BF16),
            pltpu.VMEM((B, 2, SQ, D), F32),
            pltpu.VMEM((B, SQ, 2 * D), BF16),
            pltpu.SemaphoreType.DMA((NBUF, 4)),
            pltpu.SemaphoreType.DMA((2, 4)),
            pltpu.SemaphoreType.DMA((2,)),
            pltpu.SemaphoreType.DMA((B,)),
        ],
        compiler_params=pltpu.CompilerParams(vmem_limit_bytes=96 * 1024 * 1024, disable_bounds_checks=True),
    )(A_x, B_x, A_wq, B_wq, A_wo, B_wo, t(A_k_cache), t(A_v_cache), t(B_k_cache), t(B_v_cache))
```

```python
import math
import jax
import jax.numpy as jnp
from jax import lax
import jax.experimental.pallas as pl
import jax.experimental.pallas.tpu as pltpu

B, SQ, D = 8, 128, 640
H, SK, DH = 32, 1024, 192
HP = H // 2
P2 = 2 * DH
NSTEP = HP * B
NBUF = 4
NCH = 12
OFF = 4
LAG = 5
CUT = 640
FIRST = 48
PER = 10
WQ_ROWS = D // B
WO_ROWS = P2 // B
QSCALE = (DH ** -0.5) * math.log2(math.e)
NT = (((1,), (1,)), ((), ()))
F32 = jnp.float32
BF16 = jnp.bfloat16


def _queues():
    groups = []
    for i in range(12):
        g = [(32 * i + 8, 8, CUT, SK - CUT), (32 * i + 16, 24 if i < 11 else 16, 0, SK)]
        if i < 11:
            g.append((32 * i + 40, 8, 0, CUT))
        groups.append(g)
    head = [(0, 8, 0, SK), (8, 8, 0, CUT)]
    q0 = [(j, p) for g in groups[6:] + [head] for j in range(4) for p in g]
    q1 = [(j, p) for g in groups[:6] for j in range(4) for p in g]

    def split(q):
        return [q[len(q) * c // NCH:len(q) * (c + 1) // NCH] for c in range(NCH)]
    return split(q0), split(q1)


QCH = _queues()


def _kernel(xa, xb, wqa, wqb, woa, wob, kta, vta, ktb, vtb, o_hbm,
            x_v, wq_v, wo_v, kv_v, q_v, acc_v, out_v, sem_kv, sem_w, sem_x, sem_o):
    kv_hbm = (kta, vta, ktb, vtb)

    def start(cp, prio):
        src, dst, sem = cp
        pltpu.make_async_copy(src, dst, sem).start(priority=prio)

    def pair(p0, p1, c0=None, c1=None):
        for n in range(max(len(p0), len(p1))):
            for prio, lst, cond in ((0, p0, c0), (1, p1, c1)):
                if n < len(lst):
                    if cond is None:
                        start(lst[n], prio)
                    else:
                        pl.when(cond)(lambda cp=lst[n], prio=prio: start(cp, prio))

    def wait_all(buf, sem):
        pltpu.make_async_copy(buf, buf, sem).wait()

    def kv_copies(t, queue, c):
        slot = t % NBUF
        tb = t % B
        th = t // B
        return [(kv_hbm[j].at[tb, th, pl.ds(r, nr), pl.ds(c0, nc)],
                 kv_v.at[slot, j, pl.ds(r, nr), pl.ds(c0, nc)], sem_kv.at[slot, j])
                for j, (r, nr, c0, nc) in QCH[queue][c]]

    def wq_piece(hp, j, br):
        c0 = pl.multiple_of(hp * P2, 128)
        rq = pl.multiple_of(j * WQ_ROWS, 16)
        return ((wqa, wqb)[br].at[pl.ds(rq, WQ_ROWS), pl.ds(c0, P2)], wq_v.at[hp, br, pl.ds(rq, WQ_ROWS)],
                sem_w.at[hp % 2, br])

    def wo_piece(hp, j, br):
        ro = pl.multiple_of(j * WO_ROWS, 16)
        r0 = pl.multiple_of(hp * P2 + j * WO_ROWS, 16)
        return ((woa, wob)[br].at[pl.ds(r0, WO_ROWS)], wo_v.at[hp, br, pl.ds(ro, WO_ROWS)],
                sem_w.at[hp % 2, 2 + br])

    def o_copy(b):
        return pltpu.make_async_copy(out_v.at[b], o_hbm.at[b], sem_o.at[b])

    lane = lax.broadcasted_iota(jnp.int32, (SQ, 128), 1) < 64
    ones = jnp.ones((16, SK), BF16)

    def qproj(br, b, hp):
        q = jnp.dot(x_v[b, br], wq_v[hp, br], preferred_element_type=F32) * QSCALE
        t0, t1, t2 = q[:, :128], q[:, 128:256], q[:, 256:]
        q_v[b, br, 0] = jnp.concatenate([t0, jnp.where(lane, t1, 0.0)], axis=1).astype(BF16)
        q_v[b, br, 1] = jnp.concatenate([jnp.where(lane, 0.0, t1), t2], axis=1).astype(BF16)

    def qk(slot, b, br, hh):
        return jnp.dot(q_v[b, br, hh], kv_v[slot, 2 * br, pl.ds(hh * 128, 256), :], preferred_element_type=F32)

    def sm(s):
        m = jnp.max(s, axis=1, keepdims=True)
        return jnp.exp2(s - m).astype(BF16)

    def pv(slot, p, br, hh):
        va = jnp.concatenate([kv_v[slot, 2 * br + 1, pl.ds(hh * DH, DH), :], ones], axis=0)
        ot = lax.dot_general(va, p, NT, preferred_element_type=F32)
        inv = 1.0 / ot[DH:DH + 1, :]
        return (ot[:DH] * inv).astype(BF16)

    def oproj(b, hp, br, o1, o2):
        op = jnp.concatenate([o1, o2], axis=0).T
        acc_v[b, br] += jnp.dot(op, wo_v[hp, br], preferred_element_type=F32)

    def oproj_final(b, hp, br, o1, o2):
        op = jnp.concatenate([o1, o2], axis=0).T
        r = acc_v[b, br] + jnp.dot(op, wo_v[hp, br], preferred_element_type=F32)
        out_v[b, :, pl.ds(br * D, D)] = r.astype(BF16)

    def wait_wo(hp):
        for br in range(2):
            wait_all(wo_v.at[hp, br], sem_w.at[hp % 2, 2 + br])

    def x_pieces(b):
        return [((xa, xb)[br].at[b, pl.ds(r, 32)], x_v.at[b, br, pl.ds(r, 32)], sem_x.at[b])
                for r in range(0, SQ, 32) for br in range(2)]

    l0, l1 = [], []
    x01 = x_pieces(0) + x_pieces(1)
    for j in range(B):
        l0 += [wq_piece(0, j, 0), wq_piece(0, j, 1)] + x01[2 * j:2 * j + 2]
    for b in range(2, B):
        l0 += x_pieces(b)
    k0 = [cp for c in range(NCH) for cp in kv_copies(0, 1, c)] + [cp for c in range(NCH) for cp in kv_copies(0, 0, c)]
    for j in range(B):
        l1 += [wo_piece(0, j, 0), wo_piece(0, j, 1), wq_piece(1, j, 0), wq_piece(1, j, 1)] + k0[6 * j:6 * j + 6]
    n1 = 48 + (len(k0) - 48) // 2
    l1 += k0[48:n1]
    l0 += k0[n1:]
    for c in range(NCH - OFF):
        l0 += kv_copies(1, 0, c)
        l1 += kv_copies(1, 1, c)
    for k in range(2):
        l1 += [wq_piece(2, k, 0), wq_piece(2, k, 1), wo_piece(1, k, 0), wo_piece(1, k, 1)]
    pair(l0[:FIRST], l1[:FIRST])
    acc_v[...] = jnp.zeros(acc_v.shape, F32)
    for br in range(2):
        wait_all(wq_v.at[0, br], sem_w.at[0, br])

    def q0(b, carry):
        wait_all(x_v.at[b], sem_x.at[b])
        qproj(0, b, 0)
        qproj(1, b, 0)
        for k in range(B):
            @pl.when(b == k)
            def _():
                lo = FIRST + PER * k
                pair(l0[lo:lo + PER], l1[lo:lo + PER])
        return carry

    lax.fori_loop(0, B, q0, 0)
    lo = FIRST + PER * B
    pair(l0[lo:], l1[lo:])

    def step(t, carry):
        hp = t // B
        b = t % B
        slot = t % NBUF
        tp = t + 2
        hq = jnp.minimum(tp // B + 2, HP - 1)
        ho = jnp.minimum(tp // B + 1, HP - 1)

        @pl.when(b == 0)
        def _():
            for br in range(2):
                wait_all(wq_v.at[hp + 1, br], sem_w.at[(hp + 1) % 2, br])
            wait_wo(hp)

        for j in range(4):
            wait_all(kv_v.at[slot, j], sem_kv.at[slot, j])

        def chunk(c):
            s, cc = divmod(2 * NCH + c - OFF, NCH)
            pair(kv_copies(t + s, 0, cc), kv_copies(t + s, 1, cc))

        def fetch_wq(br):
            pair([], [wq_piece(hq, tp % B, br)], c1=tp < NSTEP - 2 * B)

        def fetch_wo(br):
            pair([], [wo_piece(ho, tp % B, br)], c1=tp < NSTEP - B)

        sa1 = qk(slot, b, 0, 0)
        chunk(0)
        sa2 = qk(slot, b, 0, 1)
        chunk(1)
        oa1 = pv(slot, sm(sa1), 0, 0)
        chunk(2)
        sb1 = qk(slot, b, 1, 0)
        chunk(3)
        oa2 = pv(slot, sm(sa2), 0, 1)
        chunk(4)
        sb2 = qk(slot, b, 1, 1)
        chunk(5)
        ob1 = pv(slot, sm(sb1), 1, 0)
        chunk(6)
        fetch_wo(0)
        oproj(b, hp, 0, oa1, oa2)
        chunk(7)
        ob2 = pv(slot, sm(sb2), 1, 1)
        chunk(8)
        fetch_wq(0)
        qproj(0, b, hp + 1)
        chunk(9)
        fetch_wo(1)
        oproj(b, hp, 1, ob1, ob2)
        chunk(10)
        fetch_wq(1)
        qproj(1, b, hp + 1)
        chunk(11)
        return carry

    lax.fori_loop(0, NSTEP - B, step, 0)

    wait_wo(HP - 1)

    def tail_step(t, carry):
        b = t % B
        slot = t % NBUF

        @pl.when(t == NSTEP - 1)
        def _():
            for bb in range(B - 1):
                o_copy(bb).start(priority=1)

        for j in range(4):
            wait_all(kv_v.at[slot, j], sem_kv.at[slot, j])

        def chunk(c):
            s1, c1 = divmod(2 * NCH + c - OFF, NCH)
            s0, c0 = divmod(2 * NCH + c - OFF - LAG, NCH)
            ok0 = t + s0 < NSTEP
            if c < LAG:
                ok0 = jnp.logical_and(ok0, t > NSTEP - B)
            pair(kv_copies(jnp.minimum(t + s0, NSTEP - 1), 0, c0), kv_copies(jnp.minimum(t + s1, NSTEP - 1), 1, c1),
                 ok0, t + s1 < NSTEP)

        sa1 = qk(slot, b, 0, 0)
        chunk(0)
        sa2 = qk(slot, b, 0, 1)
        chunk(1)
        oa1 = pv(slot, sm(sa1), 0, 0)
        chunk(2)
        sb1 = qk(slot, b, 1, 0)
        chunk(3)
        chunk(4)
        oa2 = pv(slot, sm(sa2), 0, 1)
        chunk(5)
        sb2 = qk(slot, b, 1, 1)
        chunk(6)
        ob1 = pv(slot, sm(sb1), 1, 0)
        chunk(7)
        chunk(8)
        oproj_final(b, HP - 1, 0, oa1, oa2)
        chunk(9)
        ob2 = pv(slot, sm(sb2), 1, 1)
        chunk(10)
        chunk(11)
        oproj_final(b, HP - 1, 1, ob1, ob2)
        return carry

    lax.fori_loop(NSTEP - B, NSTEP, tail_step, 0)

    o_copy(B - 1).start()
    for b in range(B):
        o_copy(b).wait()


@jax.jit
def pallas_concat_heads__mha_block_cached__gqa_block_cached__near_ridge_kernel(
    A_x, A_k_cache, A_v_cache, A_wq, A_wo, B_x, B_k_cache, B_v_cache, B_wq, B_wo):
    t = lambda z: jnp.swapaxes(z, 2, 3).reshape(B, HP, P2, SK)
    any_spec = pl.BlockSpec(memory_space=pl.ANY)
    return pl.pallas_call(
        _kernel,
        in_specs=[any_spec] * 10,
        out_specs=any_spec,
        out_shape=jax.ShapeDtypeStruct((B, SQ, 2 * D), BF16),
        scratch_shapes=[
            pltpu.VMEM((B, 2, SQ, D), BF16),
            pltpu.VMEM((HP, 2, D, P2), BF16),
            pltpu.VMEM((HP, 2, P2, D), BF16),
            pltpu.VMEM((NBUF, 4, P2, SK), BF16),
            pltpu.VMEM((B, 2, 2, SQ, 256), BF16),
            pltpu.VMEM((B, 2, SQ, D), F32),
            pltpu.VMEM((B, SQ, 2 * D), BF16),
            pltpu.SemaphoreType.DMA((NBUF, 4)),
            pltpu.SemaphoreType.DMA((2, 4)),
            pltpu.SemaphoreType.DMA((B,)),
            pltpu.SemaphoreType.DMA((B,)),
        ],
        compiler_params=pltpu.CompilerParams(vmem_limit_bytes=96 * 1024 * 1024, disable_bounds_checks=True,
                                             disable_semaphore_checks=True),
    )(A_x, B_x, A_wq, B_wq, A_wo, B_wo, t(A_k_cache), t(A_v_cache), t(B_k_cache), t(B_v_cache))
```

```python
import math

import jax
import jax.numpy as jnp
from jax import lax
import jax.experimental.pallas as pl
import jax.experimental.pallas.tpu as pltpu

B, SQ, D = 8, 128, 640
H, SK, DH = 32, 1024, 192
HP = H // 2
P2 = 2 * DH
NSTEP = HP * B
NBUF = 4
NCH = 12
OFF = 4
LAG = 5
CUT = 640
FIRST = 48
PER = 10
WQ_BANDS = 10
WO_ROWS = P2 // B
SCALE = (DH ** -0.5) * math.log2(math.e)
NT = (((1,), (1,)), ((), ()))
F32 = jnp.float32
BF16 = jnp.bfloat16


def _queues():
    groups = [[(0, 8, 0, SK), (8, 8, 0, CUT)]]
    for i in range(12):
        g = [(32 * i + 8, 8, CUT, SK - CUT), (32 * i + 16, 24 if i < 11 else 16, 0, SK)]
        if i < 11:
            g.append((32 * i + 40, 8, 0, CUT))
        groups.append(g)

    def split(gs):
        q = [(j, p) for g in gs for j in range(4) for p in g]
        return [q[len(q) * c // NCH:len(q) * (c + 1) // NCH] for c in range(NCH)]

    return split(groups[7:]), split(groups[:7])


QCH = _queues()


def _kernel(xa, xb, wqa, wqb, woa, wob, kta, vta, ktb, vtb, o_hbm,
            x_v, wq_v, wo_v, kv_v, q_v, acc_v, out_v, sem_kv, sem_w, sem_x, sem_o):
    kv_hbm = (kta, vta, ktb, vtb)

    def start(cp, prio):
        src, dst, sem = cp
        pltpu.make_async_copy(src, dst, sem).start(priority=prio)

    def pair(p0, p1, c0=None, c1=None):
        for n in range(max(len(p0), len(p1))):
            for prio, lst, cond in ((0, p0, c0), (1, p1, c1)):
                if n < len(lst):
                    if cond is None:
                        start(lst[n], prio)
                    else:
                        pl.when(cond)(lambda cp=lst[n], prio=prio: start(cp, prio))

    def wait_all(buf, sem):
        pltpu.make_async_copy(buf, buf, sem).wait()

    def kv_copies(t, queue, c):
        slot = t % NBUF
        tb = t % B
        th = t // B
        return [(kv_hbm[j].at[tb, th, pl.ds(r, nr), pl.ds(c0, nc)],
                 kv_v.at[slot, j, pl.ds(r, nr), pl.ds(c0, nc)], sem_kv.at[slot, j])
                for j, (r, nr, c0, nc) in QCH[queue][c]]

    def wait_kv(slot):
        for j in range(4):
            wait_all(kv_v.at[slot, j], sem_kv.at[slot, j])

    def wq_piece(hp, j, br):
        c0 = pl.multiple_of(hp * P2, 128)
        r = pl.multiple_of(j * 8, 8)
        return ((wqa, wqb)[br].at[:, pl.ds(r, 8), pl.ds(c0, P2)], wq_v.at[hp, br, :, pl.ds(r, 8)],
                sem_w.at[hp % 2, br])

    def wo_piece(hp, j, br):
        r = pl.multiple_of(j * WO_ROWS, 16)
        r0 = pl.multiple_of(hp * P2 + j * WO_ROWS, 16)
        return ((woa, wob)[br].at[pl.ds(r0, WO_ROWS)], wo_v.at[hp, br, pl.ds(r, WO_ROWS)],
                sem_w.at[hp % 2, 2 + br])

    def wait_wq(hp):
        for br in range(2):
            wait_all(wq_v.at[hp, br], sem_w.at[hp % 2, br])

    def wait_wo(hp):
        for br in range(2):
            wait_all(wo_v.at[hp, br], sem_w.at[hp % 2, 2 + br])

    def x_pieces(b):
        return [((xa, xb)[br].at[b, pl.ds(r, 32)], x_v.at[b, br, pl.ds(r, 32)], sem_x.at[b])
                for r in range(0, SQ, 32) for br in range(2)]

    def o_half(br):
        cols = pl.ds(br * D, D)
        return out_v.at[B - 1, :, cols], o_hbm.at[B - 1, :, cols], sem_o.at[B - 1]

    lane = lax.broadcasted_iota(jnp.int32, (SQ, 128), 1) < 64
    ones = jnp.ones((16, SK), BF16)

    def qproj(br, b, hp):
        q = jnp.dot(x_v[b, br], wq_v[hp, br].reshape(D, P2), preferred_element_type=F32)
        t0, t1, t2 = q[:, :128], q[:, 128:256], q[:, 256:]
        q_v[b, br, 0] = jnp.concatenate([t0, jnp.where(lane, t1, 0.0)], axis=1).astype(BF16)
        q_v[b, br, 1] = jnp.concatenate([jnp.where(lane, 0.0, t1), t2], axis=1).astype(BF16)

    def qk(slot, b, br, hh):
        return jnp.dot(q_v[b, br, hh], kv_v[slot, 2 * br, pl.ds(hh * 128, 256), :],
                       preferred_element_type=F32)

    def sm(s):
        m = jnp.max(s, axis=1, keepdims=True)
        return jnp.exp2((s - m) * SCALE).astype(BF16)

    def pv(slot, p, br, hh):
        va = jnp.concatenate([kv_v[slot, 2 * br + 1, pl.ds(hh * DH, DH), :], ones], axis=0)
        ot = lax.dot_general(va, p, NT, preferred_element_type=F32)
        inv = 1.0 / ot[DH:DH + 1, :]
        return (ot[:DH] * inv).astype(BF16)

    def oproj(b, hp, br, o1, o2):
        op = jnp.concatenate([o1, o2], axis=0).T
        return acc_v[b, br] + jnp.dot(op, wo_v[hp, br], preferred_element_type=F32)

    l0, l1 = [], []
    x01 = x_pieces(0) + x_pieces(1)
    for j in range(B):
        l0 += [wq_piece(0, j, 0), wq_piece(0, j, 1)] + x01[2 * j:2 * j + 2]
    for b in range(2, B):
        l0 += x_pieces(b)
    k0 = [cp for queue in (1, 0) for c in range(NCH) for cp in kv_copies(0, queue, c)]
    for j in range(B):
        l1 += [wo_piece(0, j, 0), wo_piece(0, j, 1), wq_piece(1, j, 0), wq_piece(1, j, 1)]
        l1 += k0[6 * j:6 * j + 6]
    n1 = 6 * B + (len(k0) - 6 * B) // 2
    l1 += k0[6 * B:n1]
    l0 += k0[n1:]
    for c in range(NCH - OFF):
        l0 += kv_copies(1, 0, c)
        l1 += kv_copies(1, 1, c)
    for k in range(2):
        l1 += [wq_piece(2, k, 0), wq_piece(2, k, 1), wo_piece(1, k, 0), wo_piece(1, k, 1)]
    pair(l0[:FIRST], l1[:FIRST])
    acc_v[...] = jnp.zeros(acc_v.shape, F32)
    wait_wq(0)

    def first_q(b, carry):
        wait_all(x_v.at[b], sem_x.at[b])
        qproj(0, b, 0)
        qproj(1, b, 0)
        for k in range(B):
            @pl.when(b == k)
            def _():
                lo = FIRST + PER * k
                pair(l0[lo:lo + PER], l1[lo:lo + PER])
        return carry

    lax.fori_loop(0, B, first_q, 0)
    pair(l0[FIRST + PER * B:], l1[FIRST + PER * B:])

    def step(t, carry):
        hp = t // B
        b = t % B
        slot = t % NBUF
        tp = t + 2
        hq = jnp.minimum(tp // B + 2, HP - 1)
        ho = jnp.minimum(tp // B + 1, HP - 1)

        @pl.when(b == 0)
        def _():
            wait_wq(hp + 1)
            wait_wo(hp)

        wait_kv(slot)

        def chunk(c):
            s, cc = divmod(2 * NCH + c - OFF, NCH)
            pair(kv_copies(t + s, 0, cc), kv_copies(t + s, 1, cc))

        def fetch(cp, n, ok):
            src, dst, sem = cp
            lo, hi = pl.ds(0, n), pl.ds(n, n)
            pair([(src.at[lo], dst.at[lo], sem)], [(src.at[hi], dst.at[hi], sem)], ok, ok)

        def fetch_wq(br):
            fetch(wq_piece(hq, tp % B, br), WQ_BANDS // 2, tp < NSTEP - 2 * B)

        def fetch_wo(br):
            fetch(wo_piece(ho, tp % B, br), WO_ROWS // 2, tp < NSTEP - B)

        sa1 = qk(slot, b, 0, 0)
        chunk(0)
        sa2 = qk(slot, b, 0, 1)
        chunk(1)
        oa1 = pv(slot, sm(sa1), 0, 0)
        chunk(2)
        sb1 = qk(slot, b, 1, 0)
        chunk(3)
        oa2 = pv(slot, sm(sa2), 0, 1)
        chunk(4)
        sb2 = qk(slot, b, 1, 1)
        chunk(5)
        ob1 = pv(slot, sm(sb1), 1, 0)
        chunk(6)
        fetch_wo(0)
        acc_v[b, 0] = oproj(b, hp, 0, oa1, oa2)
        chunk(7)
        ob2 = pv(slot, sm(sb2), 1, 1)
        chunk(8)
        fetch_wq(0)
        qproj(0, b, hp + 1)
        chunk(9)
        fetch_wo(1)
        acc_v[b, 1] = oproj(b, hp, 1, ob1, ob2)
        chunk(10)
        fetch_wq(1)
        qproj(1, b, hp + 1)
        chunk(11)
        return carry

    lax.fori_loop(0, NSTEP - B, step, 0)

    wait_wo(HP - 1)

    def tail_step(t, carry):
        b = t % B
        slot = t % NBUF

        wait_kv(slot)

        @pl.when(t == NSTEP - 1)
        def _():
            n = 0
            for r in range(0, SQ, 16):
                for bb in range(B - 1):
                    rows = pl.ds(r, 16)
                    start((out_v.at[bb, rows], o_hbm.at[bb, rows], sem_o.at[bb]), n % 2)
                    n += 1

        def chunk(c):
            s1, c1 = divmod(2 * NCH + c - OFF, NCH)
            s0, c0 = divmod(2 * NCH + c - OFF - LAG, NCH)
            ok0 = t + s0 < NSTEP
            if c < LAG:
                ok0 = jnp.logical_and(ok0, t > NSTEP - B)
            pair(kv_copies(jnp.minimum(t + s0, NSTEP - 1), 0, c0),
                 kv_copies(jnp.minimum(t + s1, NSTEP - 1), 1, c1),
                 ok0, t <= NSTEP - 1 - s1)

        sa1 = qk(slot, b, 0, 0)
        chunk(0)
        sa2 = qk(slot, b, 0, 1)
        chunk(1)
        oa1 = pv(slot, sm(sa1), 0, 0)
        chunk(2)
        sb1 = qk(slot, b, 1, 0)
        chunk(3)
        chunk(4)
        oa2 = pv(slot, sm(sa2), 0, 1)
        chunk(5)
        sb2 = qk(slot, b, 1, 1)
        chunk(6)
        ob1 = pv(slot, sm(sb1), 1, 0)
        chunk(7)
        chunk(8)
        chunk(9)
        ob2 = pv(slot, sm(sb2), 1, 1)
        chunk(10)
        chunk(11)
        out_v[b, :, pl.ds(0, D)] = oproj(b, HP - 1, 0, oa1, oa2).astype(BF16)

        @pl.when(t == NSTEP - 1)
        def _():
            start(o_half(0), 0)

        out_v[b, :, pl.ds(D, D)] = oproj(b, HP - 1, 1, ob1, ob2).astype(BF16)
        return carry

    lax.fori_loop(NSTEP - B, NSTEP, tail_step, 0)

    start(o_half(1), 0)
    for b in range(B):
        pltpu.make_async_copy(out_v.at[b], o_hbm.at[b], sem_o.at[b]).wait()


@jax.jit
def pallas_concat_heads__mha_block_cached__gqa_block_cached__near_ridge_kernel(
    A_x: jax.Array,
    A_k_cache: jax.Array,
    A_v_cache: jax.Array,
    A_wq: jax.Array,
    A_wo: jax.Array,
    B_x: jax.Array,
    B_k_cache: jax.Array,
    B_v_cache: jax.Array,
    B_wq: jax.Array,
    B_wo: jax.Array,
):
    def kv(z):
        return jnp.swapaxes(z, 2, 3).reshape(B, HP, P2, SK)

    def wq(z):
        return z.reshape(WQ_BANDS, D // WQ_BANDS, H * DH)

    any_spec = pl.BlockSpec(memory_space=pl.ANY)
    return pl.pallas_call(
        _kernel,
        in_specs=[any_spec] * 10,
        out_specs=any_spec,
        out_shape=jax.ShapeDtypeStruct((B, SQ, 2 * D), BF16),
        scratch_shapes=[
            pltpu.VMEM((B, 2, SQ, D), BF16),
            pltpu.VMEM((HP, 2, WQ_BANDS, D // WQ_BANDS, P2), BF16),
            pltpu.VMEM((HP, 2, P2, D), BF16),
            pltpu.VMEM((NBUF, 4, P2, SK), BF16),
            pltpu.VMEM((B, 2, 2, SQ, 256), BF16),
            pltpu.VMEM((B, 2, SQ, D), F32),
            pltpu.VMEM((B, SQ, 2 * D), BF16),
            pltpu.SemaphoreType.DMA((NBUF, 4)),
            pltpu.SemaphoreType.DMA((2, 4)),
            pltpu.SemaphoreType.DMA((B,)),
            pltpu.SemaphoreType.DMA((B,)),
        ],
        compiler_params=pltpu.CompilerParams(
            vmem_limit_bytes=96 * 1024 * 1024,
            disable_bounds_checks=True,
            disable_semaphore_checks=True,
        ),
    )(A_x, B_x, wq(A_wq), wq(B_wq), A_wo, B_wo,
      kv(A_k_cache), kv(A_v_cache), kv(B_k_cache), kv(B_v_cache))
```
